```python
import os as _os
_os.environ.setdefault("JAX_PLATFORMS", "cpu")
import jax
import jax.numpy as jnp

def _softmax(x, axis=-1):
    return jax.nn.softmax(x, axis=axis)
def _gelu(x):
    return jax.nn.gelu(x, approximate=True)
def _silu(x):
    return jax.nn.silu(x)
def _sigmoid(x):
    return jax.nn.sigmoid(x)
def _layernorm(x, axis=-1, eps=1e-5):
    m = jnp.mean(x, axis=axis, keepdims=True)
    v = jnp.var(x, axis=axis, keepdims=True)
    return (x - m) / jnp.sqrt(v + eps)
def _scatter_add(tgt, idx, src, axis=0):
    return tgt.at[idx].add(src)
def _segment_sum(src, seg, n):
    return jax.ops.segment_sum(src, seg, n)
class _Rng:
    def __init__(self, key):
        self._k = key
    def _next(self):
        self._k, sub = jax.random.split(self._k)
        return sub
    def normal(self, shape):
        return jax.random.normal(self._next(), shape, dtype=jnp.bfloat16)
    def randint(self, lo, hi, shape):
        return jax.random.randint(self._next(), shape, lo, hi, dtype=jnp.int32)
    def uniform(self, shape, lo=0.0, hi=1.0):
        return jax.random.uniform(self._next(), shape, jnp.bfloat16, lo, hi)
    def permutation(self, n):
        return jax.random.permutation(self._next(), n)


kernel_name = 'sequential_preLN__linear_attn_block__glu_gated_reglu__prompt'

def setup_inputs():
    _rng = _Rng(jax.random.key(int.from_bytes(__import__("os").urandom(4), "little")))
    _w = (lambda a: (lambda t: t.astype(jnp.bfloat16) if jnp.issubdtype(t.dtype, jnp.floating) else t)(jnp.asarray(a)))
    def _A_setup():
        B, S, D = 1, 2048, 640
        return {
            "x": _w((lambda *s: _rng.normal(s) * 0.05)(B, S, D)),
            "wqkv": _w((lambda *s: _rng.normal(s) * 0.05)(D, 3 * D)),
            "wo": _w((lambda *s: _rng.normal(s) * 0.05)(D, D)),
        }
    _A_in = _A_setup()

    def _B_setup():
        B, S, D, F = 1, 2048, 640, 1536
        return {
            "x": _w((lambda *s: _rng.normal(s) * 0.05)(B, S, D)),
            "W_gate": _w((lambda *s: _rng.normal(s) * 0.05)(D, F) * (2.0 / D) ** 0.5),
            "W_up": _w((lambda *s: _rng.normal(s) * 0.05)(D, F) * (2.0 / D) ** 0.5),
            "W_down": _w((lambda *s: _rng.normal(s) * 0.05)(F, D) * (1.0 / F) ** 0.5),
        }
    _B_in = _B_setup()

    return {
        "A_x": _A_in["x"],
        "A_wqkv": _A_in["wqkv"],
        "A_wo": _A_in["wo"],
        "B_x": _B_in["x"],
        "B_W_gate": _B_in["W_gate"],
        "B_W_up": _B_in["W_up"],
        "B_W_down": _B_in["W_down"],
    }

def reference(A_x, A_wqkv, A_wo, B_x, B_W_gate, B_W_up, B_W_down):
    def _A_ref(x, wqkv, wo):
        B, S, D = x.shape
        H = 32; Dh = D // H
        qkv = (lambda x, *d: x.transpose(*d))((x @ wqkv).reshape(B, S, 3, H, Dh), 2, 0, 3, 1, 4)
        q, k, v = qkv[0], qkv[1], qkv[2]
        phi = lambda t: jnp.where(t > 0, t + 1, jnp.exp(t)) + 1e-6
        pq, pk = phi(q), phi(k)
        kv = jnp.einsum("bhsd,bhse->bhde", pk, v)
        z = jnp.einsum("bhsd->bhd", pk)
        num = jnp.einsum("bhqd,bhde->bhqe", pq, kv)
        den = jnp.einsum("bhqd,bhd->bhq", pq, z)[..., None] + 1e-6
        o = num / den
        return (lambda x, *d: x.transpose(*d))(o, 0, 2, 1, 3).reshape(B, S, D) @ wo

    def _B_ref(x, W_gate, W_up, W_down):
        gate = jnp.einsum("bsd,df->bsf", x, W_gate)
        up = jnp.einsum("bsd,df->bsf", x, W_up)
        gate = gate * (lambda x, dt: x.astype(dt))(gate > 0, gate.dtype)
        h = gate * up
        return jnp.einsum("bsf,fd->bsd", h, W_down)

    x = A_x
    h = x + _A_ref(_layernorm(x, axis=-1), A_wqkv, A_wo)
    h2 = h + _B_ref(_layernorm(h, axis=-1), B_W_gate, B_W_up, B_W_down)
    return h2
```

```python
import functools
import jax
import jax.numpy as jnp
from jax import lax
import jax.experimental.pallas as pl
import jax.experimental.pallas.tpu as pltpu

S, D, H, DH, F = 2048, 640, 32, 20, 1536
TS = 512
NT = S // TS
KVROWS = 160
KVSTART = (0, 112, 240, 368, 480)
NT_DIMS = (((1,), (1,)), ((), ()))


def _ln(x):
    m = jnp.mean(x, axis=-1, keepdims=True)
    xc = x - m
    v = jnp.mean(xc * xc, axis=-1, keepdims=True)
    return xc * lax.rsqrt(v + 1e-5)


def _phi(t):
    return jnp.where(t > 0, t + 1.0, jnp.exp(t)) + 1e-6


def _kernel(x_hbm, wqkv_hbm, wo_hbm, wg_hbm, wu_hbm, wd_hbm, out_hbm,
            x_v, wqkv_v, wo_v, wg_v, wu_v, wd_v, xn_v, wkT_v, kv_v, z_v, m_v, mb_v,
            zmat_v, e_v, out_v, sem_x, sem_w, sem_o):
    f32, bf16 = jnp.float32, jnp.bfloat16

    def x_copy(i):
        return pltpu.make_async_copy(x_hbm.at[pl.ds(i * TS, TS), :], x_v.at[pl.ds(i * TS, TS), :], sem_x.at[i])

    def out_copy(i):
        return pltpu.make_async_copy(out_v.at[pl.ds(i * TS, TS), :], out_hbm.at[pl.ds(i * TS, TS), :], sem_o.at[i])

    c_wk = pltpu.make_async_copy(wqkv_hbm.at[:, pl.ds(D, D)], wqkv_v.at[:, pl.ds(D, D)], sem_w.at[0])
    c_wv = pltpu.make_async_copy(wqkv_hbm.at[:, pl.ds(2 * D, D)], wqkv_v.at[:, pl.ds(2 * D, D)], sem_w.at[1])
    c_wq = pltpu.make_async_copy(wqkv_hbm.at[:, pl.ds(0, D)], wqkv_v.at[:, pl.ds(0, D)], sem_w.at[2])
    c_wo = pltpu.make_async_copy(wo_hbm, wo_v, sem_w.at[3])
    c_wg = pltpu.make_async_copy(wg_hbm, wg_v, sem_w.at[4])
    c_wu = pltpu.make_async_copy(wu_hbm, wu_v, sem_w.at[5])
    c_wd = pltpu.make_async_copy(wd_hbm, wd_v, sem_w.at[6])

    c_wk.start()
    x_copy(0).start()
    c_wv.start()
    for i in range(1, NT):
        x_copy(i).start()
    c_wo.start()
    c_wq.start()
    c_wg.start()
    c_wu.start()
    c_wd.start()

    kv_v[...] = jnp.zeros(kv_v.shape, f32)
    z_v[...] = jnp.zeros(z_v.shape, f32)
    m_v[...] = jnp.zeros(m_v.shape, f32)

    c_wk.wait()
    wkT_v[...] = wqkv_v[:, pl.ds(D, D)].T
    c_wv.wait()

    def phase1(i, carry):
        x_copy(i).wait()
        r0 = pl.multiple_of(i * TS, TS)
        xn = _ln(x_v[pl.ds(r0, TS), :].astype(f32)).astype(bf16)
        xn_v[pl.ds(r0, TS), :] = xn
        v = jnp.dot(xn, wqkv_v[:, pl.ds(2 * D, D)], preferred_element_type=f32).astype(bf16)
        kT = lax.dot_general(wkT_v[...], xn, NT_DIMS, preferred_element_type=f32)
        pkT = _phi(kT)
        zs = pkT[:, 0:128]
        for c in range(1, TS // 128):
            zs = zs + pkT[:, c * 128:(c + 1) * 128]
        z_v[...] += zs
        pkTb = pkT.astype(bf16)
        for j in range(5):
            s0 = KVSTART[j]
            kv_v[j] += jnp.dot(pkTb[s0:s0 + KVROWS, :], v[:, j * 128:(j + 1) * 128],
                               preferred_element_type=f32)
        return carry

    lax.fori_loop(0, NT, phase1, 0)

    c_wo.wait()
    for j in range(5):
        s0 = KVSTART[j]
        dh = (lax.broadcasted_iota(jnp.int32, (KVROWS, 128), 0) + s0) // DH
        eh = (lax.broadcasted_iota(jnp.int32, (KVROWS, 128), 1) + j * 128) // DH
        kvm = jnp.where(dh == eh, kv_v[j], 0.0).astype(bf16)
        m_v[pl.ds(s0, KVROWS), :] += jnp.dot(kvm, wo_v[pl.ds(j * 128, 128), :], preferred_element_type=f32)
    mb_v[...] = m_v[...].astype(bf16)
    zcol = jnp.sum(z_v[...], axis=-1, keepdims=True)
    dh = lax.broadcasted_iota(jnp.int32, (D, 128), 0) // DH
    ln = lax.broadcasted_iota(jnp.int32, (D, 128), 1)
    zmat_v[...] = jnp.where((ln & 31) == dh, jnp.where(ln < 64, zcol, 0.0), 0.0).astype(bf16)
    er = lax.broadcasted_iota(jnp.int32, (128, D), 0)
    ec = lax.broadcasted_iota(jnp.int32, (128, D), 1) // DH
    e_v[...] = jnp.where(((er & 31) == ec) & (er < 64), 1.0, 0.0).astype(bf16)

    c_wq.wait()
    c_wg.wait()
    c_wu.wait()
    c_wd.wait()

    def phase2(i, carry):
        r0 = pl.multiple_of(i * TS, TS)
        xn = xn_v[pl.ds(r0, TS), :]
        q = jnp.dot(xn, wqkv_v[:, pl.ds(0, D)], preferred_element_type=f32)
        pq = _phi(q)
        den = jnp.dot(pq.astype(bf16), zmat_v[...], preferred_element_type=f32) + 1e-6
        r = 1.0 / den
        r_hi = r.astype(bf16)
        r_lo = (r - r_hi.astype(f32)).astype(bf16)
        lane = lax.broadcasted_iota(jnp.int32, (TS, 128), 1)
        r2 = jnp.where(lane < 32, r_hi, r_lo)
        rexp = jnp.dot(r2, e_v[...], preferred_element_type=f32)
        a = jnp.dot((pq * rexp).astype(bf16), mb_v[...], preferred_element_type=f32)
        h = x_v[pl.ds(r0, TS), :].astype(f32) + a
        hn = _ln(h).astype(bf16)
        g = jnp.dot(hn, wg_v[...], preferred_element_type=f32)
        u = jnp.dot(hn, wu_v[...], preferred_element_type=f32)
        hh = (jnp.maximum(g, 0.0) * u).astype(bf16)
        o = h + jnp.dot(hh, wd_v[...], preferred_element_type=f32)
        out_v[pl.ds(r0, TS), :] = o.astype(bf16)
        out_copy(i).start()
        return carry

    lax.fori_loop(0, NT, phase2, 0)
    for i in range(NT):
        out_copy(i).wait()


@jax.jit
def pallas_sequential_preLN__linear_attn_block__glu_gated_reglu__prompt_kernel(
    A_x, A_wqkv, A_wo, B_x, B_W_gate, B_W_up, B_W_down):
    f32, bf16 = jnp.float32, jnp.bfloat16
    x = A_x.reshape(S, D)
    any_spec = pl.BlockSpec(memory_space=pl.ANY)
    out = pl.pallas_call(
        _kernel,
        out_shape=jax.ShapeDtypeStruct((S, D), bf16),
        in_specs=[any_spec] * 6,
        out_specs=any_spec,
        scratch_shapes=[
            pltpu.VMEM((S, D), bf16),
            pltpu.VMEM((D, 3 * D), bf16),
            pltpu.VMEM((D, D), bf16),
            pltpu.VMEM((D, F), bf16),
            pltpu.VMEM((D, F), bf16),
            pltpu.VMEM((F, D), bf16),
            pltpu.VMEM((S, D), bf16),
            pltpu.VMEM((D, D), bf16),
            pltpu.VMEM((5, KVROWS, 128), f32),
            pltpu.VMEM((D, 128), f32),
            pltpu.VMEM((D, D), f32),
            pltpu.VMEM((D, D), bf16),
            pltpu.VMEM((D, 128), bf16),
            pltpu.VMEM((128, D), bf16),
            pltpu.VMEM((S, D), bf16),
            pltpu.SemaphoreType.DMA((NT,)),
            pltpu.SemaphoreType.DMA((7,)),
            pltpu.SemaphoreType.DMA((NT,)),
        ],
        compiler_params=pltpu.CompilerParams(vmem_limit_bytes=100 * 1024 * 1024),
    )(x, A_wqkv, A_wo, B_W_gate, B_W_up, B_W_down)
    return out.reshape(1, S, D)
```

```python
import jax
import jax.numpy as jnp
from jax import lax
import jax.experimental.pallas as pl
import jax.experimental.pallas.tpu as pltpu

S, D, H, DH, F = 2048, 640, 32, 20, 1536
TS = 256
NT = S // TS
KVROWS = 160
KVSTART = (0, 112, 240, 368, 480)
NT_DIMS = (((1,), (1,)), ((), ()))


def _ln(x):
    m = jnp.mean(x, axis=-1, keepdims=True)
    xc = x - m
    v = jnp.mean(xc * xc, axis=-1, keepdims=True)
    return xc * lax.rsqrt(v + 1e-5)


def _phi(t):
    return jnp.where(t > 0, t + 1.0, jnp.exp(t)) + 1e-6


def _kernel(x_hbm, wqkv_hbm, wo_hbm, wg_hbm, wu_hbm, wd_hbm, out_hbm,
            x_v, wqkv_v, wo_v, wg_v, wu_v, wd_v, xn_v, wkT_v, g_v, z_v, m_v, mb_v,
            wqT_v, wqp_v, zp_v, zrow_v, out_v, h_v, hn_v, gate_v, pk_v, sem_x, sem_w, sem_o, sem_l):
    f32, bf16 = jnp.float32, jnp.bfloat16

    def x_copy(i):
        return pltpu.make_async_copy(x_hbm.at[pl.ds(i * TS, TS), :], x_v.at[pl.ds(i * TS, TS), :], sem_x.at[i])

    def out_copy(i):
        return pltpu.make_async_copy(out_v.at[pl.ds(i * TS, TS), :], out_hbm.at[pl.ds(i * TS, TS), :], sem_o.at[i])

    c_wk = pltpu.make_async_copy(wqkv_hbm.at[:, pl.ds(D, D)], wqkv_v.at[:, pl.ds(D, D)], sem_w.at[0])
    c_wv = pltpu.make_async_copy(wqkv_hbm.at[:, pl.ds(2 * D, D)], wqkv_v.at[:, pl.ds(2 * D, D)], sem_w.at[1])
    c_wq = pltpu.make_async_copy(wqkv_hbm.at[:, pl.ds(0, D)], wqkv_v.at[:, pl.ds(0, D)], sem_w.at[2])
    c_wo = pltpu.make_async_copy(wo_hbm, wo_v, sem_w.at[3])
    c_wg = pltpu.make_async_copy(wg_hbm, wg_v, sem_w.at[4])
    c_wu = pltpu.make_async_copy(wu_hbm, wu_v, sem_w.at[5])
    c_wd = pltpu.make_async_copy(wd_hbm, wd_v, sem_w.at[6])

    c_wk.start()
    x_copy(0).start()
    x_copy(1).start()
    x_copy(2).start()
    x_copy(3).start()
    c_wq.start()
    for i in range(4, NT):
        x_copy(i).start()
    c_wv.start()
    c_wo.start()
    c_wg.start()
    c_wu.start()
    c_wd.start()

    m_v[...] = jnp.zeros(m_v.shape, f32)
    g_v[...] = jnp.zeros(g_v.shape, f32)

    def ln_x(r0):
        return _ln(x_v[pl.ds(r0, TS), :].astype(f32)).astype(bf16)

    def kt(xn):
        kT = lax.dot_general(wkT_v[...], xn, NT_DIMS, preferred_element_type=f32)
        pkT = _phi(kT)
        zs = pkT[:, 0:128]
        for c in range(1, TS // 128):
            zs = zs + pkT[:, c * 128:(c + 1) * 128]
        return pkT.astype(bf16), zs

    def gacc(r0, slot):
        g_v[...] += jnp.dot(pk_v[slot], xn_v[pl.ds(r0, TS), :], preferred_element_type=f32)

    c_wk.wait()
    wkT_v[...] = wqkv_v[:, pl.ds(D, D)].T
    x_copy(0).wait()
    x_copy(1).wait()
    xa = ln_x(0)
    xb = ln_x(TS)
    pa, za = kt(xa)
    pb, zb = kt(xb)
    pk_v[0] = pa
    pk_v[1] = pb
    z_v[...] = za + zb
    xn_v[pl.ds(0, TS), :] = xa
    xn_v[pl.ds(TS, TS), :] = xb
    c_wq.wait()

    def phase1(j, carry):
        x_copy(2 * j + 2).wait()
        x_copy(2 * j + 3).wait()
        r0 = pl.multiple_of(j * (2 * TS), 2 * TS)
        r1 = pl.multiple_of(r0 + TS, TS)
        r2 = pl.multiple_of(r0 + 2 * TS, TS)
        r3 = pl.multiple_of(r0 + 3 * TS, TS)
        xa = ln_x(r2)
        xb = ln_x(r3)
        gacc(r0, 0)
        gacc(r1, 1)
        pa, za = kt(xa)
        pb, zb = kt(xb)
        pk_v[0] = pa
        pk_v[1] = pb
        z_v[...] += za + zb
        xn_v[pl.ds(r2, TS), :] = xa
        xn_v[pl.ds(r3, TS), :] = xb
        for t in range(2):
            c0 = pl.multiple_of(jnp.minimum(2 * j + t, 4) * 128, 128)
            wqT_v[t] = wqkv_v[pl.ds(c0, 128), pl.ds(0, D)].T.astype(f32)
            for r in range(DH):
                wqp_v[pl.ds(r * H, H), pl.ds(c0, 128)] = wqT_v[t, pl.ds(r, H, stride=DH), :].astype(bf16)
        return carry

    lax.fori_loop(0, NT // 2 - 1, phase1, 0)

    c_wv.wait()
    c_wo.wait()
    c_wg.wait()
    c_wu.wait()
    c_wd.wait()
    gacc((NT - 2) * TS, 0)
    gacc((NT - 1) * TS, 1)

    def att_q(r0):
        xn = xn_v[pl.ds(r0, TS), :]
        q = lax.dot_general(xn, wqp_v[...], NT_DIMS, preferred_element_type=f32)
        return _phi(q)

    def att_r(pq):
        t = pq * zrow_v[...]
        s = t[:, 0:128]
        for j in range(1, 5):
            s = s + t[:, j * 128:(j + 1) * 128]
        s = s + pltpu.roll(s, 32, 1)
        s = s + pltpu.roll(s, 64, 1)
        r = 1.0 / (s + 1e-6)
        return jnp.concatenate([pq[:, j * 128:(j + 1) * 128] * r for j in range(5)], axis=1).astype(bf16)

    def att_h(r0, pqr):
        a = jnp.dot(pqr, mb_v[...], preferred_element_type=f32)
        h_v[pl.ds(r0, TS), :] = x_v[pl.ds(r0, TS), :].astype(f32) + a

    def ln_gate(r0):
        hn = _ln(h_v[pl.ds(r0, TS), :]).astype(bf16)
        hn_v[...] = hn
        gate_v[...] = jnp.maximum(jnp.dot(hn, wg_v[...], preferred_element_type=f32), 0.0)

    def up_hh():
        u = jnp.dot(hn_v[...], wu_v[...], preferred_element_type=f32)
        return (gate_v[...] * u).astype(bf16)

    def down(r0, hh):
        o = h_v[pl.ds(r0, TS), :] + jnp.dot(hh, wd_v[...], preferred_element_type=f32)
        out_v[pl.ds(r0, TS), :] = o.astype(bf16)

    for i in range(DH):
        zp_v[pl.ds(i * H, H), :] = z_v[pl.ds(i, H, stride=DH), :]
    zrow_v[...] = jnp.sum(zp_v[...].T, axis=0, keepdims=True)

    pq0 = att_q(0)
    kvms = []
    for j in range(5):
        s0 = KVSTART[j]
        kvj = jnp.dot(g_v[pl.ds(s0, KVROWS), :].astype(bf16), wqkv_v[:, pl.ds(2 * D + j * 128, 128)],
                      preferred_element_type=f32)
        dh = (lax.broadcasted_iota(jnp.int32, (KVROWS, 128), 0) + s0) // DH
        eh = (lax.broadcasted_iota(jnp.int32, (KVROWS, 128), 1) + j * 128) // DH
        kvms.append(jnp.where(dh == eh, kvj, 0.0).astype(bf16))
    pq1 = att_q(TS)
    for j in range(5):
        s0 = KVSTART[j]
        mj = jnp.dot(kvms[j], wo_v[pl.ds(j * 128, 128), :], preferred_element_type=f32)
        for c in range(5):
            m_v[c, pl.ds(s0, KVROWS), :] += mj[:, c * 128:(c + 1) * 128]
    for c in range(5):
        for i in range(DH):
            mb_v[pl.ds(i * H, H), pl.ds(c * 128, 128)] = m_v[c, pl.ds(i, H, stride=DH), :].astype(bf16)
    att_h(0, att_r(pq0))
    att_h(TS, att_r(pq1))
    ln_gate(0)

    def phase2(i, carry):
        r0 = pl.multiple_of(i * TS, TS)
        r1 = pl.multiple_of(i * TS + TS, TS)
        r2 = pl.multiple_of(i * TS + 2 * TS, TS)
        pq = att_q(r2)
        hh = up_hh()
        att_h(r2, att_r(pq))
        down(r0, hh)
        ln_gate(r1)
        out_copy(i).start()
        return carry

    lax.fori_loop(0, NT - 2, phase2, 0)

    down((NT - 2) * TS, up_hh())
    ln_gate((NT - 1) * TS)
    out_copy(NT - 2).start()
    hh = up_hh()
    rl = (NT - 1) * TS

    def last_copy(c):
        return pltpu.make_async_copy(out_v.at[pl.ds(rl, TS), pl.ds(c * 128, 128)],
                                     out_hbm.at[pl.ds(rl, TS), pl.ds(c * 128, 128)], sem_l.at[c])

    for c in range(5):
        o = h_v[pl.ds(rl, TS), pl.ds(c * 128, 128)] + jnp.dot(hh, wd_v[:, pl.ds(c * 128, 128)],
                                                             preferred_element_type=f32)
        out_v[pl.ds(rl, TS), pl.ds(c * 128, 128)] = o.astype(bf16)
        last_copy(c).start()
    for i in range(NT - 1):
        out_copy(i).wait()
    for c in range(5):
        last_copy(c).wait()


@jax.jit
def pallas_sequential_preLN__linear_attn_block__glu_gated_reglu__prompt_kernel(
    A_x, A_wqkv, A_wo, B_x, B_W_gate, B_W_up, B_W_down):
    f32, bf16 = jnp.float32, jnp.bfloat16
    x = A_x.reshape(S, D)
    any_spec = pl.BlockSpec(memory_space=pl.ANY)
    out = pl.pallas_call(
        _kernel,
        out_shape=jax.ShapeDtypeStruct((S, D), bf16),
        in_specs=[any_spec] * 6,
        out_specs=any_spec,
        scratch_shapes=[
            pltpu.VMEM((S, D), bf16),
            pltpu.VMEM((D, 3 * D), bf16),
            pltpu.VMEM((D, D), bf16),
            pltpu.VMEM((D, F), bf16),
            pltpu.VMEM((D, F), bf16),
            pltpu.VMEM((F, D), bf16),
            pltpu.VMEM((S, D), bf16),
            pltpu.VMEM((D, D), bf16),
            pltpu.VMEM((D, D), f32),
            pltpu.VMEM((D, 128), f32),
            pltpu.VMEM((5, D, 128), f32),
            pltpu.VMEM((D, D), bf16),
            pltpu.VMEM((2, D, 128), f32),
            pltpu.VMEM((D, D), bf16),
            pltpu.VMEM((D, 128), f32),
            pltpu.VMEM((1, D), f32),
            pltpu.VMEM((S, D), bf16),
            pltpu.VMEM((S, D), f32),
            pltpu.VMEM((TS, D), bf16),
            pltpu.VMEM((TS, F), f32),
            pltpu.VMEM((2, D, TS), bf16),
            pltpu.SemaphoreType.DMA((NT,)),
            pltpu.SemaphoreType.DMA((7,)),
            pltpu.SemaphoreType.DMA((NT,)),
            pltpu.SemaphoreType.DMA((5,)),
        ],
        compiler_params=pltpu.CompilerParams(vmem_limit_bytes=100 * 1024 * 1024),
    )(x, A_wqkv, A_wo, B_W_gate, B_W_up, B_W_down)
    return out.reshape(1, S, D)
```

```python
import jax
import jax.numpy as jnp
from jax import lax
import jax.experimental.pallas as pl
import jax.experimental.pallas.tpu as pltpu

S, D, H, DH, F = 2048, 640, 32, 20, 1536
TS = 256
NT = S // TS
KVROWS = 160
KA = 256
KVSTART = (0, 112, 240, 368, 480)
NT_DIMS = (((1,), (1,)), ((), ()))


def _ln(x):
    m = jnp.mean(x, axis=-1, keepdims=True)
    xc = x - m
    v = jnp.mean(xc * xc, axis=-1, keepdims=True)
    return xc * lax.rsqrt(v + 1e-5)


def _phi(t):
    return jnp.where(t > 0, t + 1.0, jnp.exp(t)) + 1e-6


def _kernel(x_hbm, wqkv_hbm, wo_hbm, wg_hbm, wu_hbm, wd_hbm, out_hbm,
            x_v, wqkv_v, wo_v, wg_v, wu_v, wd_v, xn_v, wkT_v, g_v, z_v, m_v, mb_v,
            wqT_v, wqp_v, zp_v, zrow_v, out_v, h_v, hn_v, gate_v, pk_v, mask_v, k_v, sem_x, sem_w, sem_o, sem_l):
    f32, bf16 = jnp.float32, jnp.bfloat16

    def x_copy(i):
        return pltpu.make_async_copy(x_hbm.at[pl.ds(i * TS, TS), :], x_v.at[pl.ds(i * TS, TS), :], sem_x.at[i])

    def out_copy(i):
        return pltpu.make_async_copy(out_v.at[pl.ds(i * TS, TS), :], out_hbm.at[pl.ds(i * TS, TS), :], sem_o.at[i])

    c_wka = pltpu.make_async_copy(wqkv_hbm.at[:, pl.ds(D, KA)], wqkv_v.at[:, pl.ds(D, KA)], sem_w.at[0])
    c_wkb = pltpu.make_async_copy(wqkv_hbm.at[:, pl.ds(D + KA, D - KA)], wqkv_v.at[:, pl.ds(D + KA, D - KA)],
                                  sem_w.at[7])
    c_wv = pltpu.make_async_copy(wqkv_hbm.at[:, pl.ds(2 * D, D)], wqkv_v.at[:, pl.ds(2 * D, D)], sem_w.at[1])
    c_wq = pltpu.make_async_copy(wqkv_hbm.at[:, pl.ds(0, D)], wqkv_v.at[:, pl.ds(0, D)], sem_w.at[2])
    c_wo = pltpu.make_async_copy(wo_hbm, wo_v, sem_w.at[3])
    c_wg = pltpu.make_async_copy(wg_hbm, wg_v, sem_w.at[4])
    c_wu = pltpu.make_async_copy(wu_hbm, wu_v, sem_w.at[5])
    c_wd = pltpu.make_async_copy(wd_hbm, wd_v, sem_w.at[6])

    x_copy(0).start()
    c_wka.start()
    x_copy(1).start()
    c_wkb.start()
    x_copy(2).start()
    x_copy(3).start()
    c_wq.start()
    for i in range(4, NT):
        x_copy(i).start()
    c_wv.start()
    c_wo.start()
    c_wg.start()
    c_wu.start()
    c_wd.start()

    m_v[...] = jnp.zeros(m_v.shape, f32)
    g_v[...] = jnp.zeros(g_v.shape, f32)
    for j in range(5):
        dh = (lax.broadcasted_iota(jnp.int32, (KVROWS, 128), 0) + KVSTART[j]) // DH
        eh = (lax.broadcasted_iota(jnp.int32, (KVROWS, 128), 1) + j * 128) // DH
        mask_v[j] = jnp.where(dh == eh, 1.0, 0.0).astype(f32)

    def ln_x(r0):
        return _ln(x_v[pl.ds(r0, TS), :].astype(f32)).astype(bf16)

    def kt(xn):
        kT = lax.dot_general(wkT_v[...], xn, NT_DIMS, preferred_element_type=f32)
        pkT = _phi(kT)
        zs = pkT[:, 0:128]
        for c in range(1, TS // 128):
            zs = zs + pkT[:, c * 128:(c + 1) * 128]
        return pkT.astype(bf16), zs

    def gacc(r0, slot):
        g_v[...] += jnp.dot(pk_v[slot], xn_v[pl.ds(r0, TS), :], preferred_element_type=f32)

    x_copy(0).wait()
    xn_v[pl.ds(0, TS), :] = ln_x(0)
    c_wka.wait()
    k_v[0] = jnp.dot(xn_v[pl.ds(0, TS), :], wqkv_v[:, pl.ds(D, KA)], preferred_element_type=f32)
    x_copy(1).wait()
    xb = ln_x(TS)
    xn_v[pl.ds(TS, TS), :] = xb
    k_v[1] = jnp.dot(xb, wqkv_v[:, pl.ds(D, KA)], preferred_element_type=f32)
    wkT_v[pl.ds(0, KA), :] = wqkv_v[:, pl.ds(D, KA)].T
    c_wkb.wait()
    k0b = jnp.dot(xn_v[pl.ds(0, TS), :], wqkv_v[:, pl.ds(D + KA, D - KA)], preferred_element_type=f32)
    wkT_v[pl.ds(KA, D - KA), :] = wqkv_v[:, pl.ds(D + KA, D - KA)].T
    k1bT = lax.dot_general(wkT_v[pl.ds(KA, D - KA), :], xn_v[pl.ds(TS, TS), :], NT_DIMS,
                           preferred_element_type=f32)
    p0 = _phi(jnp.concatenate([k_v[0], k0b], axis=1)).T
    p1 = jnp.concatenate([_phi(k_v[1]).T, _phi(k1bT)], axis=0)
    zsum = p0[:, 0:128] + p1[:, 0:128]
    for c in range(1, TS // 128):
        zsum = zsum + p0[:, c * 128:(c + 1) * 128] + p1[:, c * 128:(c + 1) * 128]
    pk_v[0] = p0.astype(bf16)
    pk_v[1] = p1.astype(bf16)
    z_v[...] = zsum
    c_wq.wait()

    def phase1(j, carry):
        x_copy(2 * j + 2).wait()
        x_copy(2 * j + 3).wait()
        r0 = pl.multiple_of(j * (2 * TS), 2 * TS)
        r1 = pl.multiple_of(r0 + TS, TS)
        r2 = pl.multiple_of(r0 + 2 * TS, TS)
        r3 = pl.multiple_of(r0 + 3 * TS, TS)
        xa = ln_x(r2)
        xb = ln_x(r3)
        gacc(r0, 0)
        gacc(r1, 1)
        pa, za = kt(xa)
        pb, zb = kt(xb)
        pk_v[0] = pa
        pk_v[1] = pb
        z_v[...] += za + zb
        xn_v[pl.ds(r2, TS), :] = xa
        xn_v[pl.ds(r3, TS), :] = xb
        for t in range(2):
            c0 = pl.multiple_of(jnp.minimum(2 * j + t, 4) * 128, 128)
            wqT_v[t] = wqkv_v[pl.ds(c0, 128), pl.ds(0, D)].T.astype(f32)
            for r in range(DH):
                wqp_v[pl.ds(r * H, H), pl.ds(c0, 128)] = wqT_v[t, pl.ds(r, H, stride=DH), :].astype(bf16)
        return carry

    lax.fori_loop(0, NT // 2 - 1, phase1, 0)

    c_wv.wait()
    c_wo.wait()
    c_wg.wait()
    c_wu.wait()
    c_wd.wait()
    gacc((NT - 2) * TS, 0)
    gacc((NT - 1) * TS, 1)

    def att_q(r0):
        xn = xn_v[pl.ds(r0, TS), :]
        q = lax.dot_general(xn, wqp_v[...], NT_DIMS, preferred_element_type=f32)
        return _phi(q)

    def att_r(pq):
        t = pq * zrow_v[...]
        s = t[:, 0:128]
        for j in range(1, 5):
            s = s + t[:, j * 128:(j + 1) * 128]
        s = s + pltpu.roll(s, 32, 1)
        s = s + pltpu.roll(s, 64, 1)
        r = 1.0 / (s + 1e-6)
        return jnp.concatenate([pq[:, j * 128:(j + 1) * 128] * r for j in range(5)], axis=1).astype(bf16)

    def att_h(r0, pqr):
        a = jnp.dot(pqr, mb_v[...], preferred_element_type=f32)
        h_v[pl.ds(r0, TS), :] = x_v[pl.ds(r0, TS), :].astype(f32) + a

    def ln_gate(r0, h=None):
        if h is None:
            h = h_v[pl.ds(r0, TS), :]
        hn = _ln(h).astype(bf16)
        hn_v[...] = hn
        gate_v[...] = jnp.maximum(jnp.dot(hn, wg_v[...], preferred_element_type=f32), 0.0)

    def up_hh():
        u = jnp.dot(hn_v[...], wu_v[...], preferred_element_type=f32)
        return (gate_v[...] * u).astype(bf16)

    def down(r0, hh):
        o = h_v[pl.ds(r0, TS), :] + jnp.dot(hh, wd_v[...], preferred_element_type=f32)
        out_v[pl.ds(r0, TS), :] = o.astype(bf16)

    for i in range(DH):
        zp_v[pl.ds(i * H, H), :] = z_v[pl.ds(i, H, stride=DH), :]
    zrow_v[...] = jnp.sum(zp_v[...].T, axis=0, keepdims=True)

    pq0 = att_q(0)
    kvms = []
    for j in range(5):
        s0 = KVSTART[j]
        kvj = jnp.dot(g_v[pl.ds(s0, KVROWS), :].astype(bf16), wqkv_v[:, pl.ds(2 * D + j * 128, 128)],
                      preferred_element_type=f32)
        kvms.append(jnp.where(mask_v[j] > 0.5, kvj, 0.0).astype(bf16))
    xn1 = xn_v[pl.ds(TS, TS), :]
    q1a = lax.dot_general(xn1, wqp_v[pl.ds(0, 256), :], NT_DIMS, preferred_element_type=f32)
    for j in range(5):
        s0 = KVSTART[j]
        mj = jnp.dot(kvms[j], wo_v[pl.ds(j * 128, 128), :], preferred_element_type=f32)
        for c in range(5):
            m_v[c, pl.ds(s0, KVROWS), :] += mj[:, c * 128:(c + 1) * 128]
    for c in range(5):
        for i in range(DH):
            mb_v[pl.ds(i * H, H), pl.ds(c * 128, 128)] = m_v[c, pl.ds(i, H, stride=DH), :].astype(bf16)
    q1b = lax.dot_general(xn1, wqp_v[pl.ds(256, 384), :], NT_DIMS, preferred_element_type=f32)
    pq1 = _phi(jnp.concatenate([q1a, q1b], axis=1))
    att_h(0, att_r(pq0))
    att_h(TS, att_r(pq1))
    ln_gate(0)

    def phase2(i, carry):
        r0 = pl.multiple_of(i * TS, TS)
        r1 = pl.multiple_of(i * TS + TS, TS)
        r2 = pl.multiple_of(i * TS + 2 * TS, TS)
        pq = att_q(r2)
        hh = up_hh()
        att_h(r2, att_r(pq))
        down(r0, hh)
        ln_gate(r1)
        out_copy(i).start()
        return carry

    lax.fori_loop(0, NT - 2, phase2, 0)

    down((NT - 2) * TS, up_hh())
    ln_gate((NT - 1) * TS)
    out_copy(NT - 2).start()
    hh = up_hh()
    rl = (NT - 1) * TS

    def last_copy(c):
        return pltpu.make_async_copy(out_v.at[pl.ds(rl, TS), pl.ds(c * 128, 128)],
                                     out_hbm.at[pl.ds(rl, TS), pl.ds(c * 128, 128)], sem_l.at[c])

    for c in range(5):
        o = h_v[pl.ds(rl, TS), pl.ds(c * 128, 128)] + jnp.dot(hh, wd_v[:, pl.ds(c * 128, 128)],
                                                             preferred_element_type=f32)
        out_v[pl.ds(rl, TS), pl.ds(c * 128, 128)] = o.astype(bf16)
        last_copy(c).start()
    for i in range(NT - 1):
        out_copy(i).wait()
    for c in range(5):
        last_copy(c).wait()


@jax.jit
def pallas_sequential_preLN__linear_attn_block__glu_gated_reglu__prompt_kernel(
    A_x, A_wqkv, A_wo, B_x, B_W_gate, B_W_up, B_W_down):
    f32, bf16 = jnp.float32, jnp.bfloat16
    x = A_x.reshape(S, D)
    any_spec = pl.BlockSpec(memory_space=pl.ANY)
    out = pl.pallas_call(
        _kernel,
        out_shape=jax.ShapeDtypeStruct((S, D), bf16),
        in_specs=[any_spec] * 6,
        out_specs=any_spec,
        scratch_shapes=[
            pltpu.VMEM((S, D), bf16),
            pltpu.VMEM((D, 3 * D), bf16),
            pltpu.VMEM((D, D), bf16),
            pltpu.VMEM((D, F), bf16),
            pltpu.VMEM((D, F), bf16),
            pltpu.VMEM((F, D), bf16),
            pltpu.VMEM((S, D), bf16),
            pltpu.VMEM((D, D), bf16),
            pltpu.VMEM((D, D), f32),
            pltpu.VMEM((D, 128), f32),
            pltpu.VMEM((5, D, 128), f32),
            pltpu.VMEM((D, D), bf16),
            pltpu.VMEM((2, D, 128), f32),
            pltpu.VMEM((D, D), bf16),
            pltpu.VMEM((D, 128), f32),
            pltpu.VMEM((1, D), f32),
            pltpu.VMEM((S, D), bf16),
            pltpu.VMEM((S, D), f32),
            pltpu.VMEM((TS, D), bf16),
            pltpu.VMEM((TS, F), f32),
            pltpu.VMEM((2, D, TS), bf16),
            pltpu.VMEM((5, KVROWS, 128), f32),
            pltpu.VMEM((2, TS, KA), f32),
            pltpu.SemaphoreType.DMA((NT,)),
            pltpu.SemaphoreType.DMA((8,)),
            pltpu.SemaphoreType.DMA((NT,)),
            pltpu.SemaphoreType.DMA((5,)),
        ],
        compiler_params=pltpu.CompilerParams(vmem_limit_bytes=100 * 1024 * 1024),
    )(x, A_wqkv, A_wo, B_W_gate, B_W_up, B_W_down)
    return out.reshape(1, S, D)
```

```python
import jax
import jax.numpy as jnp
from jax import lax
import jax.experimental.pallas as pl
import jax.experimental.pallas.tpu as pltpu

S, D, H, DH, F = 2048, 640, 32, 20, 1536
TS = 256
NT = S // TS
NC = D // 128
KA = 256
KVROWS = 160
KVSTART = (0, 112, 240, 368, 480)
NT_DIMS = (((1,), (1,)), ((), ()))


def _ln(x):
    m = jnp.mean(x, axis=-1, keepdims=True)
    xc = x - m
    v = jnp.mean(xc * xc, axis=-1, keepdims=True)
    return xc * lax.rsqrt(v + 1e-5)


def _phi(t):
    return jnp.where(t > 0, t + 1.0, jnp.exp(t)) + 1e-6


def _kernel(x_hbm, wqkv_hbm, wo_hbm, wg_hbm, wu_hbm, wd_hbm, out_hbm,
            x_v, wqkv_v, wo_v, wg_v, wu_v, wd_v, xn_v, wkT_v, g_v, z_v, m_v, mb_v,
            wqT_v, wqp_v, zp_v, zrow_v, out_v, h_v, hn_v, gate_v, pk_v, mask_v, k_v,
            sem_x, sem_w, sem_o, sem_l):
    f32, bf16 = jnp.float32, jnp.bfloat16

    def x_copy(i):
        return pltpu.make_async_copy(x_hbm.at[pl.ds(i * TS, TS), :], x_v.at[pl.ds(i * TS, TS), :],
                                     sem_x.at[i])

    def out_copy(i):
        return pltpu.make_async_copy(out_v.at[pl.ds(i * TS, TS), :], out_hbm.at[pl.ds(i * TS, TS), :],
                                     sem_o.at[i])

    def wqkv_copy(c0, n, sem):
        return pltpu.make_async_copy(wqkv_hbm.at[:, pl.ds(c0, n)], wqkv_v.at[:, pl.ds(c0, n)], sem)

    c_wka = wqkv_copy(D, KA, sem_w.at[0])
    c_wkb = wqkv_copy(D + KA, D - KA, sem_w.at[7])
    c_wv = wqkv_copy(2 * D, D, sem_w.at[1])
    c_wq = wqkv_copy(0, D, sem_w.at[2])
    c_wo = pltpu.make_async_copy(wo_hbm, wo_v, sem_w.at[3])
    c_wg = pltpu.make_async_copy(wg_hbm, wg_v, sem_w.at[4])
    c_wu = pltpu.make_async_copy(wu_hbm, wu_v, sem_w.at[5])
    c_wd = pltpu.make_async_copy(wd_hbm, wd_v, sem_w.at[6])

    x_copy(0).start()
    c_wka.start()
    x_copy(1).start()
    c_wkb.start()
    x_copy(2).start()
    x_copy(3).start()
    c_wq.start()
    for i in range(4, NT):
        x_copy(i).start()
    c_wv.start()
    c_wo.start()
    c_wg.start()
    c_wu.start()
    c_wd.start()

    m_v[...] = jnp.zeros(m_v.shape, f32)
    g_v[...] = jnp.zeros(g_v.shape, f32)
    for j in range(NC):
        dh = (lax.broadcasted_iota(jnp.int32, (KVROWS, 128), 0) + KVSTART[j]) // DH
        eh = (lax.broadcasted_iota(jnp.int32, (KVROWS, 128), 1) + j * 128) // DH
        mask_v[j] = jnp.where(dh == eh, 1.0, 0.0).astype(f32)

    def ln_x(r0):
        return _ln(x_v[pl.ds(r0, TS), :].astype(f32)).astype(bf16)

    def kt(xn):
        kT = lax.dot_general(wkT_v[...], xn, NT_DIMS, preferred_element_type=f32)
        pkT = _phi(kT)
        zs = pkT[:, 0:128]
        for c in range(1, TS // 128):
            zs = zs + pkT[:, c * 128:(c + 1) * 128]
        return pkT.astype(bf16), zs

    def gacc(r0, slot):
        g_v[...] += jnp.dot(pk_v[slot], xn_v[pl.ds(r0, TS), :], preferred_element_type=f32)

    x_copy(0).wait()
    xn_v[pl.ds(0, TS), :] = ln_x(0)
    c_wka.wait()
    k_v[0] = jnp.dot(xn_v[pl.ds(0, TS), :], wqkv_v[:, pl.ds(D, KA)], preferred_element_type=f32)
    x_copy(1).wait()
    xb = ln_x(TS)
    xn_v[pl.ds(TS, TS), :] = xb
    k_v[1] = jnp.dot(xb, wqkv_v[:, pl.ds(D, KA)], preferred_element_type=f32)
    wkT_v[pl.ds(0, KA), :] = wqkv_v[:, pl.ds(D, KA)].T
    c_wkb.wait()
    k0b = jnp.dot(xn_v[pl.ds(0, TS), :], wqkv_v[:, pl.ds(D + KA, D - KA)], preferred_element_type=f32)
    wkT_v[pl.ds(KA, D - KA), :] = wqkv_v[:, pl.ds(D + KA, D - KA)].T
    k1bT = lax.dot_general(wkT_v[pl.ds(KA, D - KA), :], xn_v[pl.ds(TS, TS), :], NT_DIMS,
                           preferred_element_type=f32)
    p0 = _phi(jnp.concatenate([k_v[0], k0b], axis=1)).T
    p1 = jnp.concatenate([_phi(k_v[1]).T, _phi(k1bT)], axis=0)
    zsum = p0[:, 0:128] + p1[:, 0:128]
    for c in range(1, TS // 128):
        zsum = zsum + p0[:, c * 128:(c + 1) * 128] + p1[:, c * 128:(c + 1) * 128]
    pk_v[0] = p0.astype(bf16)
    pk_v[1] = p1.astype(bf16)
    z_v[...] = zsum
    c_wq.wait()

    def phase1(j, carry):
        x_copy(2 * j + 2).wait()
        x_copy(2 * j + 3).wait()
        r0 = pl.multiple_of(j * (2 * TS), 2 * TS)
        r1 = pl.multiple_of(r0 + TS, TS)
        r2 = pl.multiple_of(r0 + 2 * TS, TS)
        r3 = pl.multiple_of(r0 + 3 * TS, TS)
        xa = ln_x(r2)
        xb = ln_x(r3)
        gacc(r0, 0)
        gacc(r1, 1)
        pa, za = kt(xa)
        pb, zb = kt(xb)
        pk_v[0] = pa
        pk_v[1] = pb
        z_v[...] += za + zb
        xn_v[pl.ds(r2, TS), :] = xa
        xn_v[pl.ds(r3, TS), :] = xb
        for t in range(2):
            c0 = pl.multiple_of(jnp.minimum(2 * j + t, NC - 1) * 128, 128)
            wqT_v[t] = wqkv_v[pl.ds(c0, 128), pl.ds(0, D)].T.astype(f32)
            for r in range(DH):
                wqp_v[pl.ds(r * H, H), pl.ds(c0, 128)] = wqT_v[t, pl.ds(r, H, stride=DH), :].astype(bf16)
        return carry

    lax.fori_loop(0, NT // 2 - 1, phase1, 0)

    c_wv.wait()
    c_wo.wait()
    c_wg.wait()
    c_wu.wait()
    c_wd.wait()
    gacc((NT - 2) * TS, 0)
    gacc((NT - 1) * TS, 1)

    def att_q(r0):
        xn = xn_v[pl.ds(r0, TS), :]
        q = lax.dot_general(xn, wqp_v[...], NT_DIMS, preferred_element_type=f32)
        return _phi(q)

    def att_r(pq):
        t = pq * zrow_v[...]
        s = t[:, 0:128]
        for j in range(1, NC):
            s = s + t[:, j * 128:(j + 1) * 128]
        s = s + pltpu.roll(s, 32, 1)
        s = s + pltpu.roll(s, 64, 1)
        r = 1.0 / (s + 1e-6)
        return jnp.concatenate([pq[:, j * 128:(j + 1) * 128] * r for j in range(NC)], axis=1).astype(bf16)

    def att_h(r0, pqr):
        a = jnp.dot(pqr, mb_v[...], preferred_element_type=f32)
        h_v[pl.ds(r0, TS), :] = x_v[pl.ds(r0, TS), :].astype(f32) + a

    def ln_gate(r0):
        hn = _ln(h_v[pl.ds(r0, TS), :]).astype(bf16)
        hn_v[...] = hn
        gate_v[...] = jnp.maximum(jnp.dot(hn, wg_v[...], preferred_element_type=f32), 0.0)

    def up_hh():
        u = jnp.dot(hn_v[...], wu_v[...], preferred_element_type=f32)
        return (gate_v[...] * u).astype(bf16)

    def down(r0, hh):
        o = h_v[pl.ds(r0, TS), :] + jnp.dot(hh, wd_v[...], preferred_element_type=f32)
        out_v[pl.ds(r0, TS), :] = o.astype(bf16)

    for i in range(DH):
        zp_v[pl.ds(i * H, H), :] = z_v[pl.ds(i, H, stride=DH), :]
    zrow_v[...] = jnp.sum(zp_v[...].T, axis=0, keepdims=True)

    pq0 = att_q(0)
    kvms = []
    for j in range(NC):
        s0 = KVSTART[j]
        kvj = jnp.dot(g_v[pl.ds(s0, KVROWS), :].astype(bf16), wqkv_v[:, pl.ds(2 * D + j * 128, 128)],
                      preferred_element_type=f32)
        kvms.append(jnp.where(mask_v[j] > 0.5, kvj, 0.0).astype(bf16))
    xn1 = xn_v[pl.ds(TS, TS), :]
    q1a = lax.dot_general(xn1, wqp_v[pl.ds(0, 256), :], NT_DIMS, preferred_element_type=f32)
    for j in range(NC):
        s0 = KVSTART[j]
        mj = jnp.dot(kvms[j], wo_v[pl.ds(j * 128, 128), :], preferred_element_type=f32)
        for c in range(NC):
            m_v[c, pl.ds(s0, KVROWS), :] += mj[:, c * 128:(c + 1) * 128]
    for c in range(NC):
        for i in range(DH):
            mb_v[pl.ds(i * H, H), pl.ds(c * 128, 128)] = m_v[c, pl.ds(i, H, stride=DH), :].astype(bf16)
    q1b = lax.dot_general(xn1, wqp_v[pl.ds(256, D - 256), :], NT_DIMS, preferred_element_type=f32)
    pq1 = _phi(jnp.concatenate([q1a, q1b], axis=1))
    att_h(0, att_r(pq0))
    att_h(TS, att_r(pq1))
    ln_gate(0)

    def phase2(i, carry):
        r0 = pl.multiple_of(i * TS, TS)
        r1 = pl.multiple_of(i * TS + TS, TS)
        r2 = pl.multiple_of(i * TS + 2 * TS, TS)
        pq = att_q(r2)
        hh = up_hh()
        att_h(r2, att_r(pq))
        down(r0, hh)
        ln_gate(r1)
        out_copy(i).start()
        return carry

    lax.fori_loop(0, NT - 2, phase2, 0)

    down((NT - 2) * TS, up_hh())
    ln_gate((NT - 1) * TS)
    out_copy(NT - 2).start()
    hh = up_hh()
    rl = (NT - 1) * TS

    def last_copy(c):
        return pltpu.make_async_copy(out_v.at[pl.ds(rl, TS), pl.ds(c * 128, 128)],
                                     out_hbm.at[pl.ds(rl, TS), pl.ds(c * 128, 128)], sem_l.at[c])

    for c in range(NC):
        o = h_v[pl.ds(rl, TS), pl.ds(c * 128, 128)] + jnp.dot(hh, wd_v[:, pl.ds(c * 128, 128)],
                                                             preferred_element_type=f32)
        out_v[pl.ds(rl, TS), pl.ds(c * 128, 128)] = o.astype(bf16)
        last_copy(c).start()
    for i in range(NT - 1):
        out_copy(i).wait()
    for c in range(NC):
        last_copy(c).wait()


@jax.jit
def pallas_sequential_preLN__linear_attn_block__glu_gated_reglu__prompt_kernel(
    A_x, A_wqkv, A_wo, B_x, B_W_gate, B_W_up, B_W_down):
    del B_x
    f32, bf16 = jnp.float32, jnp.bfloat16
    assert A_x.shape == (1, S, D) and A_wqkv.shape == (D, 3 * D) and A_wo.shape == (D, D)
    assert B_W_gate.shape == (D, F) and B_W_up.shape == (D, F) and B_W_down.shape == (F, D)
    x = A_x.reshape(S, D)
    any_spec = pl.BlockSpec(memory_space=pl.ANY)
    out = pl.pallas_call(
        _kernel,
        out_shape=jax.ShapeDtypeStruct((S, D), bf16),
        in_specs=[any_spec] * 6,
        out_specs=any_spec,
        scratch_shapes=[
            pltpu.VMEM((S, D), bf16),
            pltpu.VMEM((D, 3 * D), bf16),
            pltpu.VMEM((D, D), bf16),
            pltpu.VMEM((D, F), bf16),
            pltpu.VMEM((D, F), bf16),
            pltpu.VMEM((F, D), bf16),
            pltpu.VMEM((S, D), bf16),
            pltpu.VMEM((D, D), bf16),
            pltpu.VMEM((D, D), f32),
            pltpu.VMEM((D, 128), f32),
            pltpu.VMEM((NC, D, 128), f32),
            pltpu.VMEM((D, D), bf16),
            pltpu.VMEM((2, D, 128), f32),
            pltpu.VMEM((D, D), bf16),
            pltpu.VMEM((D, 128), f32),
            pltpu.VMEM((1, D), f32),
            pltpu.VMEM((S, D), bf16),
            pltpu.VMEM((S, D), f32),
            pltpu.VMEM((TS, D), bf16),
            pltpu.VMEM((TS, F), f32),
            pltpu.VMEM((2, D, TS), bf16),
            pltpu.VMEM((NC, KVROWS, 128), f32),
            pltpu.VMEM((2, TS, KA), f32),
            pltpu.SemaphoreType.DMA((NT,)),
            pltpu.SemaphoreType.DMA((8,)),
            pltpu.SemaphoreType.DMA((NT,)),
            pltpu.SemaphoreType.DMA((NC,)),
        ],
        compiler_params=pltpu.CompilerParams(vmem_limit_bytes=100 * 1024 * 1024),
    )(x, A_wqkv, A_wo, B_W_gate, B_W_up, B_W_down)
    return out.reshape(1, S, D)
```
